```python
import jax
import jax.numpy as jnp

def _softmax(x, axis=-1):
    return jax.nn.softmax(x, axis=axis)
def _gelu(x):
    return jax.nn.gelu(x, approximate=True)
def _silu(x):
    return jax.nn.silu(x)
def _sigmoid(x):
    return jax.nn.sigmoid(x)
def _layernorm(x, axis=-1, eps=1e-5):
    m = jnp.mean(x, axis=axis, keepdims=True)
    v = jnp.var(x, axis=axis, keepdims=True)
    return (x - m) / jnp.sqrt(v + eps)
def _scatter_add(tgt, idx, src, axis=0):
    return tgt.at[idx].add(src)
def _segment_sum(src, seg, n):
    return jax.ops.segment_sum(src, seg, n)
class _Rng:
    def __init__(self, key):
        self._k = key
    def _next(self):
        self._k, sub = jax.random.split(self._k)
        return sub
    def normal(self, shape):
        return jax.random.normal(self._next(), shape, dtype=jnp.bfloat16)
    def randint(self, lo, hi, shape):
        return jax.random.randint(self._next(), shape, lo, hi, dtype=jnp.int32)
    def uniform(self, shape, lo=0.0, hi=1.0):
        return jax.random.uniform(self._next(), shape, jnp.bfloat16, lo, hi)
    def permutation(self, n):
        return jax.random.permutation(self._next(), n)


kernel_name = 'gated_mix__compressed_kv_cla__gqa_block_cached__decode'

def setup_inputs():
    _rng = _Rng(jax.random.key(int.from_bytes(__import__("os").urandom(4), "little")))
    _w = (lambda a: (lambda t: t.astype(jnp.bfloat16) if jnp.issubdtype(t.dtype, jnp.floating) else t)(jnp.asarray(a)))
    def _A_setup():
        B, H, Sq, Sk, D, M = 1, 32, 1, 4096, 128, 640
        Dc = 4 * D
        return {
            "x": _w((lambda *s: _rng.normal(s) * 0.05)(B, Sq, M)),
            "c_kv": _w((lambda *s: _rng.normal(s) * 0.05)(B, Sk, Dc)),
            "w_q": _w((lambda *s: _rng.normal(s) * 0.05)(M, H, D) * (M ** -0.5)),
            "w_uk": _w((lambda *s: _rng.normal(s) * 0.05)(Dc, H, D) * (Dc ** -0.5)),
            "w_uv": _w((lambda *s: _rng.normal(s) * 0.05)(Dc, H, D) * (Dc ** -0.5)),
            "w_o": _w((lambda *s: _rng.normal(s) * 0.05)(H, D, M) * ((H * D) ** -0.5)),
        }
    _A_in = _A_setup()

    def _B_setup():
        B, Sq, D = 1, 1, 640
        Hq, Hkv, Sk, Dh = 32, 32, 4096, 128
        assert Hq % Hkv == 0, (Hq, Hkv)
        return {
            "x": _w((lambda *s: _rng.normal(s) * 0.05)(B, Sq, D)),
            "k_cache": _w((lambda *s: _rng.normal(s) * 0.05)(B, Hkv, Sk, Dh)),
            "v_cache": _w((lambda *s: _rng.normal(s) * 0.05)(B, Hkv, Sk, Dh)),
            "wq": _w((lambda *s: _rng.normal(s) * 0.05)(D, Hq * Dh) * (D ** -0.5)),
            "wo": _w((lambda *s: _rng.normal(s) * 0.05)(Hq * Dh, D) * ((Hq * Dh) ** -0.5)),
        }
    _B_in = _B_setup()

    return {
        "A_x": _A_in["x"],
        "A_c_kv": _A_in["c_kv"],
        "A_w_q": _A_in["w_q"],
        "A_w_uk": _A_in["w_uk"],
        "A_w_uv": _A_in["w_uv"],
        "A_w_o": _A_in["w_o"],
        "B_x": _B_in["x"],
        "B_k_cache": _B_in["k_cache"],
        "B_v_cache": _B_in["v_cache"],
        "B_wq": _B_in["wq"],
        "B_wo": _B_in["wo"],
        "gate_w": _w((lambda *s: _rng.normal(s) * 0.05)(640)),
    }

def reference(A_x, A_c_kv, A_w_q, A_w_uk, A_w_uv, A_w_o, B_x, B_k_cache, B_v_cache, B_wq, B_wo, gate_w):
    def _A_ref(x, c_kv, w_q, w_uk, w_uv, w_o):
        B, Sq, M = x.shape[0], x.shape[1], x.shape[2]
        Sk = c_kv.shape[1]
        H, D = w_q.shape[1], w_q.shape[2]
        q = jnp.einsum("bqm,mhd->bhqd", x, w_q)
        k = jnp.einsum("bkc,chd->bhkd", c_kv, w_uk)
        v = jnp.einsum("bkc,chd->bhkd", c_kv, w_uv)
        scores = jnp.einsum("bhqd,bhkd->bhqk", q, k) * (D ** -0.5)
        off = Sk - Sq
        qi = jnp.arange(Sq)[:, None]
        kj = jnp.arange(Sk)[None, :]
        cmask = kj <= (qi + off)
        scores = jnp.where(cmask[None, None], scores, -1e9)
        p = _softmax(scores, axis=-1)
        ctx = jnp.einsum("bhqk,bhkd->bhqd", p, v)
        return jnp.einsum("bhqd,hdm->bqm", ctx, w_o)

    def _B_ref(x, k_cache, v_cache, wq, wo):
        B, Sq, D = x.shape
        Hq, Dh = 32, 128
        Hkv = k_cache.shape[1]
        rep = Hq // Hkv
        q = (lambda x, *d: x.transpose(*d))((x @ wq).reshape(B, Sq, Hq, Dh), 0, 2, 1, 3)
        k = jnp.repeat(k_cache, rep, axis=1)
        v = jnp.repeat(v_cache, rep, axis=1)
        scores = jnp.einsum("bhqd,bhkd->bhqk", q, k) * (Dh ** -0.5)
        p = _softmax(scores, axis=-1)
        o = jnp.einsum("bhqk,bhkd->bhqd", p, v)
        return (lambda x, *d: x.transpose(*d))(o, 0, 2, 1, 3).reshape(B, Sq, Hq * Dh) @ wo

    x = A_x
    g = _sigmoid((x * gate_w).sum(-1, keepdims=True))
    a = _A_ref(x, A_c_kv, A_w_q, A_w_uk, A_w_uv, A_w_o)
    b = _B_ref(x, B_k_cache, B_v_cache, B_wq, B_wo)
    return g * a + (1 - g) * b
```

```python
import functools
import contextlib
import jax
import jax.numpy as jnp
from jax import lax
import jax.experimental.pallas as pl
import jax.experimental.pallas.tpu as pltpu

F32 = jnp.float32
BF16 = jnp.bfloat16
H, D, M, SK, DC = 32, 128, 640, 4096, 512


def _nt(a, b):
    return lax.dot_general(a, b, (((1,), (1,)), ((), ())), preferred_element_type=F32)


def _nn(a, b):
    return jnp.dot(a, b, preferred_element_type=F32)


def _iota(shape, dim):
    return lax.broadcasted_iota(jnp.int32, shape, dim)


def make_kernel(scopes=False, HC=4, MR=16):
    scope = jax.named_scope if scopes else (lambda n: contextlib.nullcontext())
    NG = H // HC
    S_X, S_G, S_WQ, S_WUK, S_CKV, S_WUV, S_BWQ = range(7)
    S_K = 7
    S_WO = S_K + 2 * NG
    S_BWO = S_WO + 1
    BWO_CH = [(0, 2048), (2048, 1024), (3072, 512), (3584, 256), (3840, 128), (3968, 128)]
    NSEM = S_BWO + len(BWO_CH)

    def kernel(x_h, ckv_h, wq_h, wuk_h, wuv_h, wo_h, k_h, v_h, bwq_h, bwo_h, gw_h,
               out_ref,
               x_v, gw_v, ckv_v, wq_v, wuk_v, wuv_v, wo_v, k_v, v_v, bwq_v, bwo_v,
               vrow_s, s_s, qb_s, o_s, sems):
        def cp_x(): return pltpu.make_async_copy(x_h, x_v, sems.at[S_X])
        def cp_g(): return pltpu.make_async_copy(gw_h, gw_v, sems.at[S_G])
        def cp_wq(): return pltpu.make_async_copy(wq_h, wq_v, sems.at[S_WQ])
        def cp_wuk(): return pltpu.make_async_copy(wuk_h, wuk_v, sems.at[S_WUK])
        def cp_ckv(): return pltpu.make_async_copy(ckv_h.at[0], ckv_v, sems.at[S_CKV])
        def cp_wuv(): return pltpu.make_async_copy(wuv_h, wuv_v, sems.at[S_WUV])
        def cp_bwq(): return pltpu.make_async_copy(bwq_h, bwq_v, sems.at[S_BWQ])
        def cp_k(g): return pltpu.make_async_copy(k_h.at[0, pl.ds(g * HC, HC)], k_v.at[pl.ds(g * HC, HC)], sems.at[S_K + 2 * g])
        def cp_v(g): return pltpu.make_async_copy(v_h.at[0, pl.ds(g * HC, HC)], v_v.at[pl.ds(g * HC, HC)], sems.at[S_K + 2 * g + 1])
        def cp_wo(): return pltpu.make_async_copy(wo_h, wo_v, sems.at[S_WO])
        def cp_bwo(j):
            s, n = BWO_CH[j]
            return pltpu.make_async_copy(bwo_h.at[pl.ds(s, n)], bwo_v.at[pl.ds(s, n)], sems.at[S_BWO + j])

        with scope("dma_start"):
            cp_x().start()
            cp_wq().start()
            cp_g().start()
            cp_wuk().start()
            cp_ckv().start()
            cp_wuv().start()
            cp_bwq().start()
            for g in range(NG):
                cp_k(g).start()
                cp_v(g).start()
            cp_wo().start()
            for j in range(len(BWO_CH)):
                cp_bwo(j).start()

        lane32 = _iota((32, 128), 1)
        row32 = _iota((32, 128), 0)

        with scope("x_prep"):
            cp_x().wait()
            xf = x_v[0].astype(F32)
            a_sel = jnp.where(_iota((160, M), 1) // 4 == _iota((160, M), 0),
                              jnp.broadcast_to(xf, (160, M)), 0.0).astype(BF16)
            r_sel = (_iota((M, 128), 0) % 4 == _iota((M, 128), 1) // 32).astype(F32).astype(BF16)
            vrow_s[...] = _nn(a_sel, r_sel)

        with scope("qA_wait"):
            cp_wq().wait()
        with scope("qA"):
            adiag = (lane32 % 32) == (31 - row32)
            UN = 4

            def qa_body(it, acc):
                for tt in range(UN):
                    t = it * UN + tt
                    vt = vrow_s[pl.ds(t, 1), :]
                    lhs = jnp.where(adiag, jnp.broadcast_to(vt, (32, 128)), 0.0).astype(BF16)
                    tile = wq_v[pl.ds(4 * t, 4)].reshape(128, 128)
                    acc = acc + _nn(lhs, tile)
                return acc

            qa = lax.fori_loop(0, 160 // UN, qa_body, jnp.zeros((32, 128), F32))
            qa_b = qa.astype(BF16)

        with scope("qabs_wait"):
            cp_wuk().wait()
        with scope("qabs"):
            skew = (lane32 + row32) % 32

            def qabs_body(u, accs):
                accs = list(accs)
                sh = (u + 97) % 128
                for cb in range(4):
                    tile = jnp.concatenate([wuk_v[128 * cb + 32 * i + u] for i in range(4)], axis=0)
                    r = _nt(qa_b, tile)
                    r = pltpu.roll(r, sh, 1)
                    accs[cb] = jnp.where(skew == u, r, accs[cb])
                return tuple(accs)

            accs = lax.fori_loop(0, 32, qabs_body, tuple(jnp.zeros((32, 128), F32) for _ in range(4)))
            qabs = jnp.concatenate([pltpu.roll(a, 0, 1, stride=1, stride_axis=0) for a in accs], axis=1)
            qabs_b = qabs.astype(BF16)

        with scope("ckv_wait"):
            cp_ckv().wait()
        with scope("attnA"):
            KC = 512
            scale = D ** -0.5

            def sc_body(c, m):
                k0 = pl.multiple_of(c * KC, KC)
                s = _nt(qabs_b, ckv_v[pl.ds(k0, KC), :]) * scale
                s_s[:, pl.ds(k0, KC)] = s
                for j in range(KC // 128):
                    m = jnp.maximum(m, s[:, 128 * j:128 * (j + 1)])
                return m

            m = lax.fori_loop(0, SK // KC, sc_body, jnp.full((32, 128), -jnp.inf, F32))
            m = jnp.max(m, axis=1, keepdims=True)

            def pv_body(c, carry):
                l, acc = carry
                k0 = pl.multiple_of(c * KC, KC)
                p = jnp.exp(s_s[:, pl.ds(k0, KC)] - m)
                for j in range(KC // 128):
                    l = l + p[:, 128 * j:128 * (j + 1)]
                acc = acc + _nn(p.astype(BF16), ckv_v[pl.ds(k0, KC), :])
                return l, acc

            l, ctxc = lax.fori_loop(0, SK // KC, pv_body,
                                    (jnp.zeros((32, 128), F32), jnp.zeros((32, DC), F32)))
            l = jnp.sum(l, axis=1, keepdims=True)
            ctxc = (ctxc / l).astype(BF16)
            jmat = (_iota((32, 128), 0) + _iota((32, 128), 1) == 31).astype(F32).astype(BF16)
            ctxc_p = jnp.concatenate([ctxc, jnp.zeros((96, DC), BF16)], axis=0)
            ctxn = _nn(jmat, ctxc_p)
            ctxk = [pltpu.roll(ctxn[:, 128 * cb:128 * (cb + 1)], 0, 1, stride=1, stride_axis=0) for cb in range(4)]

        with scope("wuv_wait"):
            cp_wuv().wait()
        with scope("ctxA"):
            diag = (lane32 % 32) == row32

            def cx_body(u, acc):
                sh = (128 - u) % 128
                for cb in range(4):
                    lhs = jnp.where(diag, pltpu.roll(ctxk[cb], sh, 1), 0.0).astype(BF16)
                    tile = jnp.concatenate([wuv_v[128 * cb + 32 * i + u] for i in range(4)], axis=0)
                    acc = acc + _nn(lhs, tile)
                return acc

            ctx = lax.fori_loop(0, 32, cx_body, jnp.zeros((32, 128), F32))
            ctx_b = ctx.astype(BF16)

        with scope("bwq_wait"):
            cp_bwq().wait()
        with scope("qB"):
            xb = jnp.broadcast_to(xf, (MR, M)).astype(BF16)
            for n in range(4096 // 512):
                qb_s[:, 512 * n:512 * (n + 1)] = _nn(xb, bwq_v[:, 512 * n:512 * (n + 1)]).astype(BF16)

        scale = D ** -0.5

        def head_body(h, _):
            @pl.when(h % HC == 0)
            def _():
                g = h // HC
                cp_k(g).wait()
                cp_v(g).wait()
            c0 = pl.multiple_of(h * 128, 128)
            q = qb_s[:, pl.ds(c0, 128)]
            s = _nt(q, k_v[h]) * scale
            mm = jnp.max(s, axis=1, keepdims=True)
            p = jnp.exp(s - mm)
            l = jnp.sum(p, axis=1, keepdims=True)
            o = _nn(p.astype(BF16), v_v[h])
            o_s[:, pl.ds(c0, 128)] = (o / l).astype(BF16)
            return 0

        with scope("attnB"):
            lax.fori_loop(0, H, head_body, 0)

        with scope("wo_wait"):
            cp_wo().wait()
        with scope("outA"):
            acc_a = jnp.zeros((16, M), F32)
            row16 = _iota((16, 128), 0)
            for h in range(H):
                grp = ctx_b[16 * (h // 16):16 * (h // 16 + 1), :]
                lhs = jnp.where(row16 == (h % 16), grp, jnp.zeros_like(grp))
                acc_a = acc_a + _nn(lhs, wo_v[h])
            a = jnp.sum(acc_a, axis=0, keepdims=True)

        with scope("gate"):
            cp_g().wait()
            gw = gw_v[...].astype(F32).reshape(1, M)
            gate = jax.nn.sigmoid(jnp.sum(xf * gw, axis=1, keepdims=True))

        with scope("outB"):
            acc_b = jnp.zeros((MR, M), F32)
            for j, (s0, n) in enumerate(BWO_CH):
                cp_bwo(j).wait()
                acc_b = acc_b + _nn(o_s[:, s0:s0 + n], bwo_v[s0:s0 + n, :])
            b = acc_b[0:1, :]
            out = gate * a + (1.0 - gate) * b
            out_ref[0] = out.astype(BF16)

    return kernel, NSEM


def build(scopes=False, **kw):
    kernel, NSEM = make_kernel(scopes=scopes, **kw)
    MR = kw.get("MR", 16)
    hbm = pl.BlockSpec(memory_space=pl.ANY)

    def fn(A_x, A_c_kv, A_w_q, A_w_uk, A_w_uv, A_w_o, B_x, B_k_cache, B_v_cache, B_wq, B_wo, gate_w):
        return pl.pallas_call(
            kernel,
            out_shape=jax.ShapeDtypeStruct((1, 1, M), BF16),
            in_specs=[hbm] * 11,
            out_specs=pl.BlockSpec(memory_space=pltpu.VMEM),
            scratch_shapes=[
                pltpu.VMEM((1, 1, M), BF16),
                pltpu.VMEM((M,), BF16),
                pltpu.VMEM((SK, DC), BF16),
                pltpu.VMEM((M, H, D), BF16),
                pltpu.VMEM((DC, H, D), BF16),
                pltpu.VMEM((DC, H, D), BF16),
                pltpu.VMEM((H, D, M), BF16),
                pltpu.VMEM((H, SK, D), BF16),
                pltpu.VMEM((H, SK, D), BF16),
                pltpu.VMEM((M, H * D), BF16),
                pltpu.VMEM((H * D, M), BF16),
                pltpu.VMEM((160, 128), F32),
                pltpu.VMEM((32, SK), F32),
                pltpu.VMEM((MR, 4096), BF16),
                pltpu.VMEM((MR, 4096), BF16),
                pltpu.SemaphoreType.DMA((NSEM,)),
            ],
            compiler_params=pltpu.CompilerParams(vmem_limit_bytes=112 * 1024 * 1024),
        )(A_x, A_c_kv, A_w_q, A_w_uk, A_w_uv, A_w_o, B_k_cache, B_v_cache, B_wq, B_wo, gate_w)
    return fn


_KERNEL_FN = None


@jax.jit
def pallas_gated_mix__compressed_kv_cla__gqa_block_cached__decode_kernel(
    A_x: jax.Array,
    A_c_kv: jax.Array,
    A_w_q: jax.Array,
    A_w_uk: jax.Array,
    A_w_uv: jax.Array,
    A_w_o: jax.Array,
    B_x: jax.Array,
    B_k_cache: jax.Array,
    B_v_cache: jax.Array,
    B_wq: jax.Array,
    B_wo: jax.Array,
    gate_w: jax.Array,
):
    return build()(A_x, A_c_kv, A_w_q, A_w_uk, A_w_uv, A_w_o, B_x, B_k_cache, B_v_cache, B_wq, B_wo, gate_w)
```

```python
import jax
import jax.numpy as jnp
from jax import lax
import jax.experimental.pallas as pl
import jax.experimental.pallas.tpu as pltpu

F32 = jnp.float32
BF16 = jnp.bfloat16

H = 32
D = 128
M = 640
SK = 4096
DC = 512
QR = 8

V_SPLIT = (0, 12, 20, 26, 32)
BWO_CHUNKS = ((0, 3072), (3072, 512), (3584, 256), (3840, 128), (3968, 128))

S_X, S_G, S_WQ, S_WUK, S_CKV, S_WUV, S_BWQ, S_K, S_WO = range(9)
S_V = 9
S_BWO = S_V + len(V_SPLIT) - 1
N_SEM = S_BWO + len(BWO_CHUNKS)


def _nt(a, b):
    return lax.dot_general(a, b, (((1,), (1,)), ((), ())), preferred_element_type=F32)


def _nn(a, b):
    return jnp.dot(a, b, preferred_element_type=F32)


def _iota(shape, dim):
    return lax.broadcasted_iota(jnp.int32, shape, dim)


def _kernel(x_h, ckv_h, wq_h, wuk_h, wuv_h, wo_h, k_h, v_h, bwq_h, bwo_h, gw_h,
            out_ref,
            x_v, gw_v, ckv_v, wq_v, wuk_v, wuv_v, wo_v, k_v, v_v, bwq_v, bwo_v,
            vrow_s, s_s, qb_s, o_s, acc_s, sems):
    def whole(src, dst, slot):
        return pltpu.make_async_copy(src, dst, sems.at[slot])

    cp_x = whole(x_h, x_v, S_X)
    cp_g = whole(gw_h, gw_v, S_G)
    cp_wq = whole(wq_h, wq_v, S_WQ)
    cp_wuk = whole(wuk_h, wuk_v, S_WUK)
    cp_ckv = whole(ckv_h.at[0], ckv_v, S_CKV)
    cp_wuv = whole(wuv_h, wuv_v, S_WUV)
    cp_bwq = whole(bwq_h, bwq_v, S_BWQ)
    cp_k = whole(k_h.at[0], k_v, S_K)
    cp_wo = whole(wo_h, wo_v, S_WO)
    cp_v = [whole(v_h.at[0, pl.ds(lo, hi - lo)], v_v.at[pl.ds(lo, hi - lo)], S_V + g)
            for g, (lo, hi) in enumerate(zip(V_SPLIT[:-1], V_SPLIT[1:]))]
    cp_bwo = [whole(bwo_h.at[pl.ds(s0, n)], bwo_v.at[pl.ds(s0, n)], S_BWO + j)
              for j, (s0, n) in enumerate(BWO_CHUNKS)]

    for cp in [cp_wq, cp_x, cp_wuk, cp_ckv, cp_wuv, cp_bwq, cp_k, *cp_v, cp_wo, cp_g, *cp_bwo]:
        cp.start()

    lane = _iota((32, 128), 1)
    row = _iota((32, 128), 0)
    scale = D ** -0.5

    cp_x.wait()
    xf = x_v[0].astype(F32)
    a_sel = jnp.where(_iota((160, M), 1) // 4 == _iota((160, M), 0),
                      jnp.broadcast_to(xf, (160, M)), 0.0).astype(BF16)
    r_sel = (_iota((M, 128), 0) % 4 == _iota((M, 128), 1) // 32).astype(F32).astype(BF16)
    vrow_s[...] = _nn(a_sel, r_sel)

    cp_wq.wait()
    anti_diag = (lane % 32) == (31 - row)
    unroll = 4

    def q_body(it, acc):
        for tt in range(unroll):
            t = it * unroll + tt
            xt = jnp.broadcast_to(vrow_s[pl.ds(t, 1), :], (32, 128))
            lhs = jnp.where(anti_diag, xt, 0.0).astype(BF16)
            tile = wq_v[pl.ds(4 * t, 4)].reshape(128, 128)
            acc = acc + _nn(lhs, tile)
        return acc

    qa = lax.fori_loop(0, 160 // unroll, q_body, jnp.zeros((32, 128), F32))
    qa_b = qa.astype(BF16)

    cp_wuk.wait()
    skew = (lane + row) % 32

    def qabs_body(u, accs):
        accs = list(accs)
        shift = (u + 97) % 128
        for cb in range(4):
            tile = jnp.concatenate([wuk_v[128 * cb + 32 * i + u] for i in range(4)], axis=0)
            r = pltpu.roll(_nt(qa_b, tile), shift, 1)
            accs[cb] = jnp.where(skew == u, r, accs[cb])
        return tuple(accs)

    accs = lax.fori_loop(0, 32, qabs_body, tuple(jnp.zeros((32, 128), F32) for _ in range(4)))
    qabs_b = jnp.concatenate(
        [pltpu.roll(a, 0, 1, stride=1, stride_axis=0) for a in accs], axis=1).astype(BF16)

    cp_ckv.wait()
    kc = 512

    def score_body(c, m):
        k0 = pl.multiple_of(c * kc, kc)
        s = _nt(qabs_b, ckv_v[pl.ds(k0, kc), :]) * scale
        s_s[:, pl.ds(k0, kc)] = s
        for j in range(kc // 128):
            m = jnp.maximum(m, s[:, 128 * j:128 * (j + 1)])
        return m

    m = lax.fori_loop(0, SK // kc, score_body, jnp.full((32, 128), -jnp.inf, F32))
    m = jnp.max(m, axis=1, keepdims=True)

    def pv_body(c, carry):
        l, acc = carry
        k0 = pl.multiple_of(c * kc, kc)
        p = jnp.exp(s_s[:, pl.ds(k0, kc)] - m)
        for j in range(kc // 128):
            l = l + p[:, 128 * j:128 * (j + 1)]
        return l, acc + _nn(p.astype(BF16), ckv_v[pl.ds(k0, kc), :])

    l, ctxc = lax.fori_loop(0, SK // kc, pv_body,
                            (jnp.zeros((32, 128), F32), jnp.zeros((32, DC), F32)))
    ctxc = (ctxc / jnp.sum(l, axis=1, keepdims=True)).astype(BF16)
    flip = (_iota((32, 128), 0) + _iota((32, 128), 1) == 31).astype(F32).astype(BF16)
    ctxn = _nn(flip, jnp.concatenate([ctxc, jnp.zeros((96, DC), BF16)], axis=0))
    ctxk = [pltpu.roll(ctxn[:, 128 * cb:128 * (cb + 1)], 0, 1, stride=1, stride_axis=0)
            for cb in range(4)]

    cp_wuv.wait()
    diag = (lane % 32) == row

    def ctx_body(u, acc):
        shift = (128 - u) % 128
        for cb in range(4):
            lhs = jnp.where(diag, pltpu.roll(ctxk[cb], shift, 1), 0.0).astype(BF16)
            tile = jnp.concatenate([wuv_v[128 * cb + 32 * i + u] for i in range(4)], axis=0)
            acc = acc + _nn(lhs, tile)
        return acc

    ctx_b = lax.fori_loop(0, 32, ctx_body, jnp.zeros((32, 128), F32)).astype(BF16)

    cp_bwq.wait()
    xb = jnp.broadcast_to(xf, (QR, M)).astype(BF16)
    for n in range(H * D // 512):
        cols = slice(512 * n, 512 * (n + 1))
        qb_s[:, cols] = _nn(xb, bwq_v[:, cols]).astype(BF16)

    cp_k.wait()

    def head_body(h, carry):
        for g, lo in enumerate(V_SPLIT[:-1]):
            @pl.when(h == lo)
            def _():
                cp_v[g].wait()
        c0 = pl.multiple_of(h * D, D)
        s = _nt(qb_s[:, pl.ds(c0, D)], k_v[h]) * scale
        p = jnp.exp(s - jnp.max(s, axis=1, keepdims=True))
        o = _nn(p.astype(BF16), v_v[h])
        o_s[:, pl.ds(c0, D)] = (o / jnp.sum(p, axis=1, keepdims=True)).astype(BF16)
        return carry

    lax.fori_loop(0, H, head_body, 0)

    cp_wo.wait()
    row16 = _iota((16, 128), 0)
    acc_a = jnp.zeros((16, M), F32)
    for h in range(H):
        grp = ctx_b[16 * (h // 16):16 * (h // 16 + 1), :]
        acc_a = acc_a + _nn(jnp.where(row16 == (h % 16), grp, jnp.zeros_like(grp)), wo_v[h])
    a = jnp.sum(acc_a, axis=0, keepdims=True)

    cp_g.wait()
    gw = gw_v[...].astype(F32).reshape(1, M)
    gate = jax.nn.sigmoid(jnp.sum(xf * gw, axis=1, keepdims=True))

    gb = jnp.broadcast_to(1.0 - gate, (8, M))
    acc_s[...] = jnp.broadcast_to(gate * a, (8, M))
    for j, (s0, n) in enumerate(BWO_CHUNKS):
        cp_bwo[j].wait()
        part = _nn(o_s[:, s0:s0 + n], bwo_v[s0:s0 + n, :])[0:8, :]
        if j + 1 < len(BWO_CHUNKS):
            acc_s[...] = acc_s[...] + gb * part
        else:
            out = acc_s[...] + gb * part
            out_ref[0] = out[0:1, :].astype(BF16)


@jax.jit
def pallas_gated_mix__compressed_kv_cla__gqa_block_cached__decode_kernel(
    A_x: jax.Array,
    A_c_kv: jax.Array,
    A_w_q: jax.Array,
    A_w_uk: jax.Array,
    A_w_uv: jax.Array,
    A_w_o: jax.Array,
    B_x: jax.Array,
    B_k_cache: jax.Array,
    B_v_cache: jax.Array,
    B_wq: jax.Array,
    B_wo: jax.Array,
    gate_w: jax.Array,
):
    del B_x
    hbm = pl.BlockSpec(memory_space=pl.ANY)
    return pl.pallas_call(
        _kernel,
        out_shape=jax.ShapeDtypeStruct((1, 1, M), BF16),
        in_specs=[hbm] * 11,
        out_specs=pl.BlockSpec(memory_space=pltpu.VMEM),
        scratch_shapes=[
            pltpu.VMEM((1, 1, M), BF16),
            pltpu.VMEM((M,), BF16),
            pltpu.VMEM((SK, DC), BF16),
            pltpu.VMEM((M, H, D), BF16),
            pltpu.VMEM((DC, H, D), BF16),
            pltpu.VMEM((DC, H, D), BF16),
            pltpu.VMEM((H, D, M), BF16),
            pltpu.VMEM((H, SK, D), BF16),
            pltpu.VMEM((H, SK, D), BF16),
            pltpu.VMEM((M, H * D), BF16),
            pltpu.VMEM((H * D, M), BF16),
            pltpu.VMEM((160, 128), F32),
            pltpu.VMEM((32, SK), F32),
            pltpu.VMEM((QR, H * D), BF16),
            pltpu.VMEM((QR, H * D), BF16),
            pltpu.VMEM((8, M), F32),
            pltpu.SemaphoreType.DMA((N_SEM,)),
        ],
        compiler_params=pltpu.CompilerParams(
            vmem_limit_bytes=112 * 1024 * 1024,
            disable_semaphore_checks=True,
        ),
    )(A_x, A_c_kv, A_w_q, A_w_uk, A_w_uv, A_w_o, B_k_cache, B_v_cache, B_wq, B_wo, gate_w)
```

```python
import jax
import jax.numpy as jnp
from jax import lax
import jax.experimental.pallas as pl
import jax.experimental.pallas.tpu as pltpu

F32 = jnp.float32
BF16 = jnp.bfloat16

H = 32
D = 128
M = 640
SK = 4096
DC = 512
QR = 8

V_SPLIT = (0, 12, 20, 26, 32)
BWO_MXU = ((0, 3072), (3072, 512), (3584, 256), (3840, 128))
BWO_VPU = ((3968, 48), (4016, 32), (4048, 32), (4080, 16))
BWO_CHUNKS = BWO_MXU + BWO_VPU
TAIL0 = BWO_VPU[0][0]

S_X, S_G, S_WQ, S_WUK, S_CKV, S_WUV, S_BWQ, S_K, S_WO = range(9)
S_V = 9
S_BWO = S_V + len(V_SPLIT) - 1
N_SEM = S_BWO + len(BWO_CHUNKS)


def _nt(a, b):
    return lax.dot_general(a, b, (((1,), (1,)), ((), ())), preferred_element_type=F32)


def _nn(a, b):
    return jnp.dot(a, b, preferred_element_type=F32)


def _iota(shape, dim):
    return lax.broadcasted_iota(jnp.int32, shape, dim)


def _kernel(x_h, ckv_h, wq_h, wuk_h, wuv_h, wo_h, k_h, v_h, bwq_h, bwo_h, gw_h,
            out_ref,
            x_v, gw_v, ckv_v, wq_v, wuk_v, wuv_v, wo_v, k_v, v_v, bwq_v, bwo_v,
            vrow_s, s_s, qb_s, o_s, acc_s, ocol_s, accv_s, sems):
    def whole(src, dst, slot):
        return pltpu.make_async_copy(src, dst, sems.at[slot])

    cp_x = whole(x_h, x_v, S_X)
    cp_g = whole(gw_h, gw_v, S_G)
    cp_wq = whole(wq_h, wq_v, S_WQ)
    cp_wuk = whole(wuk_h, wuk_v, S_WUK)
    cp_ckv = whole(ckv_h.at[0], ckv_v, S_CKV)
    cp_wuv = whole(wuv_h, wuv_v, S_WUV)
    cp_bwq = whole(bwq_h, bwq_v, S_BWQ)
    cp_k = whole(k_h.at[0], k_v, S_K)
    cp_wo = whole(wo_h, wo_v, S_WO)
    cp_v = [whole(v_h.at[0, pl.ds(lo, hi - lo)], v_v.at[pl.ds(lo, hi - lo)], S_V + g)
            for g, (lo, hi) in enumerate(zip(V_SPLIT[:-1], V_SPLIT[1:]))]
    cp_bwo = [whole(bwo_h.at[pl.ds(s0, n)], bwo_v.at[pl.ds(s0, n)], S_BWO + j)
              for j, (s0, n) in enumerate(BWO_CHUNKS)]

    for cp in [cp_wq, cp_x, cp_wuk, cp_ckv, cp_wuv, cp_bwq, cp_k, *cp_v, cp_wo, cp_g, *cp_bwo]:
        cp.start()

    lane = _iota((32, 128), 1)
    row = _iota((32, 128), 0)
    scale = D ** -0.5

    cp_x.wait()
    xf = x_v[0].astype(F32)
    a_sel = jnp.where(_iota((160, M), 1) // 4 == _iota((160, M), 0),
                      jnp.broadcast_to(xf, (160, M)), 0.0).astype(BF16)
    r_sel = (_iota((M, 128), 0) % 4 == _iota((M, 128), 1) // 32).astype(F32).astype(BF16)
    vrow_s[...] = _nn(a_sel, r_sel)

    cp_wq.wait()
    anti_diag = (lane % 32) == (31 - row)
    unroll = 4

    def q_body(it, acc):
        for tt in range(unroll):
            t = it * unroll + tt
            xt = jnp.broadcast_to(vrow_s[pl.ds(t, 1), :], (32, 128))
            lhs = jnp.where(anti_diag, xt, 0.0).astype(BF16)
            tile = wq_v[pl.ds(4 * t, 4)].reshape(128, 128)
            acc = acc + _nn(lhs, tile)
        return acc

    qa = lax.fori_loop(0, 160 // unroll, q_body, jnp.zeros((32, 128), F32))
    qa_b = qa.astype(BF16)

    cp_wuk.wait()
    skew = (lane + row) % 32

    def qabs_body(u, accs):
        accs = list(accs)
        shift = (u + 97) % 128
        for cb in range(4):
            tile = jnp.concatenate([wuk_v[128 * cb + 32 * i + u] for i in range(4)], axis=0)
            r = pltpu.roll(_nt(qa_b, tile), shift, 1)
            accs[cb] = jnp.where(skew == u, r, accs[cb])
        return tuple(accs)

    accs = lax.fori_loop(0, 32, qabs_body, tuple(jnp.zeros((32, 128), F32) for _ in range(4)))
    qabs_b = jnp.concatenate(
        [pltpu.roll(a, 0, 1, stride=1, stride_axis=0) for a in accs], axis=1).astype(BF16)

    cp_ckv.wait()
    kc = 512

    def score_body(c, m):
        k0 = pl.multiple_of(c * kc, kc)
        s = _nt(qabs_b, ckv_v[pl.ds(k0, kc), :]) * scale
        s_s[:, pl.ds(k0, kc)] = s
        for j in range(kc // 128):
            m = jnp.maximum(m, s[:, 128 * j:128 * (j + 1)])
        return m

    m = lax.fori_loop(0, SK // kc, score_body, jnp.full((32, 128), -jnp.inf, F32))
    m = jnp.max(m, axis=1, keepdims=True)

    def pv_body(c, carry):
        l, acc = carry
        k0 = pl.multiple_of(c * kc, kc)
        p = jnp.exp(s_s[:, pl.ds(k0, kc)] - m)
        for j in range(kc // 128):
            l = l + p[:, 128 * j:128 * (j + 1)]
        return l, acc + _nn(p.astype(BF16), ckv_v[pl.ds(k0, kc), :])

    l, ctxc = lax.fori_loop(0, SK // kc, pv_body,
                            (jnp.zeros((32, 128), F32), jnp.zeros((32, DC), F32)))
    ctxc = (ctxc / jnp.sum(l, axis=1, keepdims=True)).astype(BF16)
    flip = (_iota((32, 128), 0) + _iota((32, 128), 1) == 31).astype(F32).astype(BF16)
    ctxn = _nn(flip, jnp.concatenate([ctxc, jnp.zeros((96, DC), BF16)], axis=0))
    ctxk = [pltpu.roll(ctxn[:, 128 * cb:128 * (cb + 1)], 0, 1, stride=1, stride_axis=0)
            for cb in range(4)]

    cp_wuv.wait()
    diag = (lane % 32) == row

    def ctx_body(u, acc):
        shift = (128 - u) % 128
        for cb in range(4):
            lhs = jnp.where(diag, pltpu.roll(ctxk[cb], shift, 1), 0.0).astype(BF16)
            tile = jnp.concatenate([wuv_v[128 * cb + 32 * i + u] for i in range(4)], axis=0)
            acc = acc + _nn(lhs, tile)
        return acc

    ctx_b = lax.fori_loop(0, 32, ctx_body, jnp.zeros((32, 128), F32)).astype(BF16)

    cp_bwq.wait()
    xb = jnp.broadcast_to(xf, (QR, M)).astype(BF16)
    for n in range(H * D // 512):
        cols = slice(512 * n, 512 * (n + 1))
        qb_s[:, cols] = _nn(xb, bwq_v[:, cols]).astype(BF16)

    cp_k.wait()

    def head_body(h, carry):
        for g, lo in enumerate(V_SPLIT[:-1]):
            @pl.when(h == lo)
            def _():
                cp_v[g].wait()
        c0 = pl.multiple_of(h * D, D)
        s = _nt(qb_s[:, pl.ds(c0, D)], k_v[h]) * scale
        p = jnp.exp(s - jnp.max(s, axis=1, keepdims=True))
        o = _nn(p.astype(BF16), v_v[h])
        o_s[:, pl.ds(c0, D)] = (o / jnp.sum(p, axis=1, keepdims=True)).astype(BF16)
        return carry

    lax.fori_loop(0, H, head_body, 0)

    cp_wo.wait()
    row16 = _iota((16, 128), 0)
    acc_a = jnp.zeros((16, M), F32)
    for h in range(H):
        grp = ctx_b[16 * (h // 16):16 * (h // 16 + 1), :]
        acc_a = acc_a + _nn(jnp.where(row16 == (h % 16), grp, jnp.zeros_like(grp)), wo_v[h])
    a = jnp.sum(acc_a, axis=0, keepdims=True)

    cp_g.wait()
    gw = gw_v[...].astype(F32).reshape(1, M)
    gate = jax.nn.sigmoid(jnp.sum(xf * gw, axis=1, keepdims=True))

    gate_b = 1.0 - gate
    gb = jnp.broadcast_to(gate_b, (8, M))
    acc_s[...] = jnp.broadcast_to(gate * a, (8, M))
    nt = H * D - TAIL0
    o_rows = jnp.broadcast_to(o_s[0:1, TAIL0:].astype(F32), (128, nt)).astype(BF16)
    eye = (_iota((nt, nt), 0) == _iota((nt, nt), 1)).astype(F32).astype(BF16)
    ocol_s[...] = _nt(eye, o_rows) * gate_b

    for j, (s0, n) in enumerate(BWO_MXU):
        cp_bwo[j].wait()
        part = _nn(o_s[:, s0:s0 + n], bwo_v[s0:s0 + n, :])[0:8, :]
        acc_s[...] = acc_s[...] + gb * part

    sub8 = _iota((8, M), 0)
    accv_s[...] = jnp.where(sub8 == 0, acc_s[...], 0.0)
    for j, (s0, n) in enumerate(BWO_VPU):
        cp_bwo[len(BWO_MXU) + j].wait()
        oc = ocol_s[s0 - TAIL0:s0 - TAIL0 + n, :]
        outs = []
        for t in range(M // 128):
            cols = slice(128 * t, 128 * (t + 1))
            w = bwo_v[s0:s0 + n, cols].astype(F32)
            acc = accv_s[:, cols] + (w * oc).reshape(n // 8, 8, 128).sum(axis=0)
            if j + 1 < len(BWO_VPU):
                accv_s[:, cols] = acc
            else:
                outs.append(jnp.sum(acc, axis=0, keepdims=True))
        if outs:
            out_ref[0] = jnp.concatenate(outs, axis=1).astype(BF16)


@jax.jit
def pallas_gated_mix__compressed_kv_cla__gqa_block_cached__decode_kernel(
    A_x: jax.Array,
    A_c_kv: jax.Array,
    A_w_q: jax.Array,
    A_w_uk: jax.Array,
    A_w_uv: jax.Array,
    A_w_o: jax.Array,
    B_x: jax.Array,
    B_k_cache: jax.Array,
    B_v_cache: jax.Array,
    B_wq: jax.Array,
    B_wo: jax.Array,
    gate_w: jax.Array,
):
    del B_x
    hbm = pl.BlockSpec(memory_space=pl.ANY)
    return pl.pallas_call(
        _kernel,
        out_shape=jax.ShapeDtypeStruct((1, 1, M), BF16),
        in_specs=[hbm] * 11,
        out_specs=pl.BlockSpec(memory_space=pltpu.VMEM),
        scratch_shapes=[
            pltpu.VMEM((1, 1, M), BF16),
            pltpu.VMEM((M,), BF16),
            pltpu.VMEM((SK, DC), BF16),
            pltpu.VMEM((M, H, D), BF16),
            pltpu.VMEM((DC, H, D), BF16),
            pltpu.VMEM((DC, H, D), BF16),
            pltpu.VMEM((H, D, M), BF16),
            pltpu.VMEM((H, SK, D), BF16),
            pltpu.VMEM((H, SK, D), BF16),
            pltpu.VMEM((M, H * D), BF16),
            pltpu.VMEM((H * D, M), BF16),
            pltpu.VMEM((160, 128), F32),
            pltpu.VMEM((32, SK), F32),
            pltpu.VMEM((QR, H * D), BF16),
            pltpu.VMEM((QR, H * D), BF16),
            pltpu.VMEM((8, M), F32),
            pltpu.VMEM((H * D - TAIL0, 128), F32),
            pltpu.VMEM((8, M), F32),
            pltpu.SemaphoreType.DMA((N_SEM,)),
        ],
        compiler_params=pltpu.CompilerParams(
            vmem_limit_bytes=112 * 1024 * 1024,
            disable_semaphore_checks=True,
        ),
    )(A_x, A_c_kv, A_w_q, A_w_uk, A_w_uv, A_w_o, B_k_cache, B_v_cache, B_wq, B_wo, gate_w)
```

```python
import jax
import jax.numpy as jnp
from jax import lax
import jax.experimental.pallas as pl
import jax.experimental.pallas.tpu as pltpu

F32 = jnp.float32
BF16 = jnp.bfloat16

H = 32
D = 128
M = 640
SK = 4096
DC = 512
QR = 8

V_SPLIT = (0, 12, 20, 26, 32)
BWO_MXU = ((0, 3072), (3072, 512), (3584, 256), (3840, 128))
BWO_VPU = ((3968, 48), (4016, 32), (4048, 32), (4080, 16))
BWO_CHUNKS = BWO_MXU + BWO_VPU
TAIL0 = BWO_VPU[0][0]

S_X, S_G, S_WQ, S_WUK, S_CKV, S_WUV, S_BWQ, S_K, S_WO = range(9)
S_V = 9
S_BWO = S_V + len(V_SPLIT) - 1
N_SEM = S_BWO + len(BWO_CHUNKS)


def _nt(a, b):
    return lax.dot_general(a, b, (((1,), (1,)), ((), ())), preferred_element_type=F32)


def _nn(a, b):
    return jnp.dot(a, b, preferred_element_type=F32)


def _iota(shape, dim):
    return lax.broadcasted_iota(jnp.int32, shape, dim)


def _kernel(x_h, ckv_h, wq_h, wuk_h, wuv_h, wo_h, k_h, v_h, bwq_h, bwo_h, gw_h,
            out_ref,
            x_v, gw_v, ckv_v, wq_v, wuk_v, wuv_v, wo_v, k_v, v_v, bwq_v, bwo_v,
            vrow_s, s_s, qb_s, o_s, acc_s, ocol_s, accv_s, sems):
    def whole(src, dst, slot):
        return pltpu.make_async_copy(src, dst, sems.at[slot])

    cp_x = whole(x_h, x_v, S_X)
    cp_g = whole(gw_h, gw_v, S_G)
    cp_wq = whole(wq_h, wq_v, S_WQ)
    cp_wuk = whole(wuk_h, wuk_v, S_WUK)
    cp_ckv = whole(ckv_h.at[0], ckv_v, S_CKV)
    cp_wuv = whole(wuv_h, wuv_v, S_WUV)
    cp_bwq = whole(bwq_h, bwq_v, S_BWQ)
    cp_k = whole(k_h.at[0], k_v, S_K)
    cp_wo = whole(wo_h, wo_v, S_WO)
    cp_v = [whole(v_h.at[0, pl.ds(lo, hi - lo)], v_v.at[pl.ds(lo, hi - lo)], S_V + g)
            for g, (lo, hi) in enumerate(zip(V_SPLIT[:-1], V_SPLIT[1:]))]
    cp_bwo = [whole(bwo_h.at[pl.ds(s0, n)], bwo_v.at[pl.ds(s0, n)], S_BWO + j)
              for j, (s0, n) in enumerate(BWO_CHUNKS)]

    for cp in [cp_wq, cp_x, cp_wuk, cp_ckv, cp_wuv, cp_bwq, cp_k, *cp_v, cp_wo, cp_g, *cp_bwo]:
        cp.start()

    lane = _iota((32, 128), 1)
    row = _iota((32, 128), 0)
    scale = D ** -0.5

    cp_x.wait()
    xf = x_v[0].astype(F32)
    a_sel = jnp.where(_iota((160, M), 1) // 4 == _iota((160, M), 0),
                      jnp.broadcast_to(xf, (160, M)), 0.0).astype(BF16)
    r_sel = (_iota((M, 128), 0) % 4 == _iota((M, 128), 1) // 32).astype(F32).astype(BF16)
    vrow_s[...] = _nn(a_sel, r_sel)

    cp_wq.wait()
    anti_diag = (lane % 32) == (31 - row)
    unroll = 4

    def q_body(it, acc):
        for tt in range(unroll):
            t = it * unroll + tt
            xt = jnp.broadcast_to(vrow_s[pl.ds(t, 1), :], (32, 128))
            lhs = jnp.where(anti_diag, xt, 0.0).astype(BF16)
            tile = wq_v[pl.ds(4 * t, 4)].reshape(128, 128)
            acc = acc + _nn(lhs, tile)
        return acc

    qa = lax.fori_loop(0, 160 // unroll, q_body, jnp.zeros((32, 128), F32))
    qa_b = qa.astype(BF16)

    cp_wuk.wait()
    skew = (lane + row) % 32

    def qabs_body(u, accs):
        accs = list(accs)
        shift = (u + 97) % 128
        for cb in range(4):
            tile = jnp.concatenate([wuk_v[128 * cb + 32 * i + u] for i in range(4)], axis=0)
            r = pltpu.roll(_nt(qa_b, tile), shift, 1)
            accs[cb] = jnp.where(skew == u, r, accs[cb])
        return tuple(accs)

    accs = lax.fori_loop(0, 32, qabs_body, tuple(jnp.zeros((32, 128), F32) for _ in range(4)))
    qabs_b = jnp.concatenate(
        [pltpu.roll(a, 0, 1, stride=1, stride_axis=0) for a in accs], axis=1).astype(BF16)

    cp_ckv.wait()
    kc = 512

    def score_body(c, m):
        k0 = pl.multiple_of(c * kc, kc)
        s = _nt(qabs_b, ckv_v[pl.ds(k0, kc), :]) * scale
        s_s[:, pl.ds(k0, kc)] = s
        for j in range(kc // 128):
            m = jnp.maximum(m, s[:, 128 * j:128 * (j + 1)])
        return m

    m = lax.fori_loop(0, SK // kc, score_body, jnp.full((32, 128), -jnp.inf, F32))
    m = jnp.max(m, axis=1, keepdims=True)

    def pv_body(c, carry):
        l, acc = carry
        k0 = pl.multiple_of(c * kc, kc)
        p = jnp.exp(s_s[:, pl.ds(k0, kc)] - m)
        for j in range(kc // 128):
            l = l + p[:, 128 * j:128 * (j + 1)]
        return l, acc + _nn(p.astype(BF16), ckv_v[pl.ds(k0, kc), :])

    l, ctxc = lax.fori_loop(0, SK // kc, pv_body,
                            (jnp.zeros((32, 128), F32), jnp.zeros((32, DC), F32)))
    ctxc = (ctxc / jnp.sum(l, axis=1, keepdims=True)).astype(BF16)
    flip = (_iota((32, 128), 0) + _iota((32, 128), 1) == 31).astype(F32).astype(BF16)
    ctxn = _nn(flip, jnp.concatenate([ctxc, jnp.zeros((96, DC), BF16)], axis=0))
    ctxk = [pltpu.roll(ctxn[:, 128 * cb:128 * (cb + 1)], 0, 1, stride=1, stride_axis=0)
            for cb in range(4)]

    cp_wuv.wait()
    diag = (lane % 32) == row

    def ctx_body(u, acc):
        shift = (128 - u) % 128
        for cb in range(4):
            lhs = jnp.where(diag, pltpu.roll(ctxk[cb], shift, 1), 0.0).astype(BF16)
            tile = jnp.concatenate([wuv_v[128 * cb + 32 * i + u] for i in range(4)], axis=0)
            acc = acc + _nn(lhs, tile)
        return acc

    ctx_b = lax.fori_loop(0, 32, ctx_body, jnp.zeros((32, 128), F32)).astype(BF16)

    cp_bwq.wait()
    xb = jnp.broadcast_to(xf, (QR, M)).astype(BF16)
    for n in range(H * D // 512):
        cols = slice(512 * n, 512 * (n + 1))
        qb_s[:, cols] = _nn(xb, bwq_v[:, cols]).astype(BF16)

    cp_k.wait()

    def head_body(h, carry):
        c0 = pl.multiple_of(h * D, D)
        s = _nt(qb_s[:, pl.ds(c0, D)], k_v[h]) * scale
        p = jnp.exp(s - jnp.max(s, axis=1, keepdims=True))
        o = _nn(p.astype(BF16), v_v[h])
        o_s[:, pl.ds(c0, D)] = (o / jnp.sum(p, axis=1, keepdims=True)).astype(BF16)
        return carry

    for g, (lo, hi) in enumerate(zip(V_SPLIT[:-1], V_SPLIT[1:])):
        cp_v[g].wait()
        lax.fori_loop(lo, hi, head_body, 0)

    cp_wo.wait()
    row16 = _iota((16, 128), 0)
    acc_a = jnp.zeros((16, M), F32)
    for h in range(H):
        grp = ctx_b[16 * (h // 16):16 * (h // 16 + 1), :]
        acc_a = acc_a + _nn(jnp.where(row16 == (h % 16), grp, jnp.zeros_like(grp)), wo_v[h])
    a = jnp.sum(acc_a, axis=0, keepdims=True)

    cp_g.wait()
    gw = gw_v[...].astype(F32).reshape(1, M)
    gate = jax.nn.sigmoid(jnp.sum(xf * gw, axis=1, keepdims=True))

    gate_b = 1.0 - gate
    gb = jnp.broadcast_to(gate_b, (8, M))
    acc_s[...] = jnp.broadcast_to(gate * a, (8, M))
    nt = H * D - TAIL0
    o_rows = jnp.broadcast_to(o_s[0:1, TAIL0:].astype(F32), (128, nt)).astype(BF16)
    eye = (_iota((nt, nt), 0) == _iota((nt, nt), 1)).astype(F32).astype(BF16)
    ocol_s[...] = _nt(eye, o_rows) * gate_b

    for j, (s0, n) in enumerate(BWO_MXU):
        cp_bwo[j].wait()
        part = _nn(o_s[:, s0:s0 + n], bwo_v[s0:s0 + n, :])[0:8, :]
        acc_s[...] = acc_s[...] + gb * part

    sub8 = _iota((8, M), 0)
    accv_s[...] = jnp.where(sub8 == 0, acc_s[...], 0.0)
    for j, (s0, n) in enumerate(BWO_VPU):
        cp_bwo[len(BWO_MXU) + j].wait()
        oc = ocol_s[s0 - TAIL0:s0 - TAIL0 + n, :]
        outs = []
        for t in range(M // 128):
            cols = slice(128 * t, 128 * (t + 1))
            w = bwo_v[s0:s0 + n, cols].astype(F32)
            acc = accv_s[:, cols] + (w * oc).reshape(n // 8, 8, 128).sum(axis=0)
            if j + 1 < len(BWO_VPU):
                accv_s[:, cols] = acc
            else:
                outs.append(jnp.sum(acc, axis=0, keepdims=True))
        if outs:
            out_ref[0] = jnp.concatenate(outs, axis=1).astype(BF16)


@jax.jit
def pallas_gated_mix__compressed_kv_cla__gqa_block_cached__decode_kernel(
    A_x: jax.Array,
    A_c_kv: jax.Array,
    A_w_q: jax.Array,
    A_w_uk: jax.Array,
    A_w_uv: jax.Array,
    A_w_o: jax.Array,
    B_x: jax.Array,
    B_k_cache: jax.Array,
    B_v_cache: jax.Array,
    B_wq: jax.Array,
    B_wo: jax.Array,
    gate_w: jax.Array,
):
    del B_x
    hbm = pl.BlockSpec(memory_space=pl.ANY)
    return pl.pallas_call(
        _kernel,
        out_shape=jax.ShapeDtypeStruct((1, 1, M), BF16),
        in_specs=[hbm] * 11,
        out_specs=pl.BlockSpec(memory_space=pltpu.VMEM),
        scratch_shapes=[
            pltpu.VMEM((1, 1, M), BF16),
            pltpu.VMEM((M,), BF16),
            pltpu.VMEM((SK, DC), BF16),
            pltpu.VMEM((M, H, D), BF16),
            pltpu.VMEM((DC, H, D), BF16),
            pltpu.VMEM((DC, H, D), BF16),
            pltpu.VMEM((H, D, M), BF16),
            pltpu.VMEM((H, SK, D), BF16),
            pltpu.VMEM((H, SK, D), BF16),
            pltpu.VMEM((M, H * D), BF16),
            pltpu.VMEM((H * D, M), BF16),
            pltpu.VMEM((160, 128), F32),
            pltpu.VMEM((32, SK), F32),
            pltpu.VMEM((QR, H * D), BF16),
            pltpu.VMEM((QR, H * D), BF16),
            pltpu.VMEM((8, M), F32),
            pltpu.VMEM((H * D - TAIL0, 128), F32),
            pltpu.VMEM((8, M), F32),
            pltpu.SemaphoreType.DMA((N_SEM,)),
        ],
        compiler_params=pltpu.CompilerParams(
            vmem_limit_bytes=112 * 1024 * 1024,
            disable_semaphore_checks=True,
        ),
    )(A_x, A_c_kv, A_w_q, A_w_uk, A_w_uv, A_w_o, B_k_cache, B_v_cache, B_wq, B_wo, gate_w)
```

```python
import jax
import jax.numpy as jnp
from jax import lax
import jax.experimental.pallas as pl
import jax.experimental.pallas.tpu as pltpu

F32 = jnp.float32
BF16 = jnp.bfloat16

H = 32
D = 128
M = 640
SK = 4096
DC = 512
QR = 8

V_SPLIT = (0, 12, 20, 26, 32)
BWO_MXU = ((0, 3072), (3072, 512), (3584, 256), (3840, 128))
BWO_VPU = ((3968, 48), (4016, 32), (4048, 32), (4080, 16))
BWO_CHUNKS = BWO_MXU + BWO_VPU
TAIL0 = BWO_VPU[0][0]

S_X, S_G, S_WQ, S_WUK, S_CKV, S_WUV, S_BWQ, S_K, S_WO = range(9)
S_V = 9
S_BWO = S_V + len(V_SPLIT) - 1
N_SEM = S_BWO + len(BWO_CHUNKS)


def _nt(a, b):
    return lax.dot_general(a, b, (((1,), (1,)), ((), ())), preferred_element_type=F32)


def _nn(a, b):
    return jnp.dot(a, b, preferred_element_type=F32)


def _iota(shape, dim):
    return lax.broadcasted_iota(jnp.int32, shape, dim)


def _skew_rows(x):
    row = _iota(x.shape, 0)
    for b in range(5):
        x = jnp.where((row & (1 << b)) != 0, pltpu.roll(x, 1 << b, 1), x)
    return x


def _kernel(x_h, ckv_h, wq_h, wuk_h, wuv_h, wo_h, k_h, v_h, bwq_h, bwo_h, gw_h,
            out_ref,
            x_v, gw_v, ckv_v, wq_v, wuk_v, wuv_v, wo_v, k_v, v_v, bwq_v, bwo_v,
            vrow_s, s_s, qb_s, o_s, acc_s, ocol_s, accv_s, sems):
    def whole(src, dst, slot):
        return pltpu.make_async_copy(src, dst, sems.at[slot])

    cp_x = whole(x_h, x_v, S_X)
    cp_g = whole(gw_h, gw_v, S_G)
    cp_wq = whole(wq_h, wq_v, S_WQ)
    cp_wuk = whole(wuk_h, wuk_v, S_WUK)
    cp_ckv = whole(ckv_h.at[0], ckv_v, S_CKV)
    cp_wuv = whole(wuv_h, wuv_v, S_WUV)
    cp_bwq = whole(bwq_h, bwq_v, S_BWQ)
    cp_k = whole(k_h.at[0], k_v, S_K)
    cp_wo = whole(wo_h, wo_v, S_WO)
    cp_v = [whole(v_h.at[0, pl.ds(lo, hi - lo)], v_v.at[pl.ds(lo, hi - lo)], S_V + g)
            for g, (lo, hi) in enumerate(zip(V_SPLIT[:-1], V_SPLIT[1:]))]
    cp_bwo = [whole(bwo_h.at[pl.ds(s0, n)], bwo_v.at[pl.ds(s0, n)], S_BWO + j)
              for j, (s0, n) in enumerate(BWO_CHUNKS)]

    for cp in [cp_wq, cp_x, cp_wuk, cp_ckv, cp_wuv, cp_bwq, cp_k, *cp_v, cp_wo, cp_g, *cp_bwo]:
        cp.start()

    lane = _iota((32, 128), 1)
    row = _iota((32, 128), 0)
    scale = D ** -0.5

    cp_x.wait()
    xf = x_v[0].astype(F32)
    a_sel = jnp.where(_iota((160, M), 1) // 4 == _iota((160, M), 0),
                      jnp.broadcast_to(xf, (160, M)), 0.0).astype(BF16)
    r_sel = (_iota((M, 128), 0) % 4 == _iota((M, 128), 1) // 32).astype(F32).astype(BF16)
    vrow_s[...] = _nn(a_sel, r_sel)

    cp_wq.wait()
    anti_diag = (lane % 32) == (31 - row)
    unroll = 4

    def q_body(it, acc):
        for tt in range(unroll):
            t = it * unroll + tt
            xt = jnp.broadcast_to(vrow_s[pl.ds(t, 1), :], (32, 128))
            lhs = jnp.where(anti_diag, xt, 0.0).astype(BF16)
            tile = wq_v[pl.ds(4 * t, 4)].reshape(128, 128)
            acc = acc + _nn(lhs, tile)
        return acc

    qa = lax.fori_loop(0, 160 // unroll, q_body, jnp.zeros((32, 128), F32))
    qa_b = qa.astype(BF16)

    cp_wuk.wait()
    skew = (lane + row) % 32

    def qabs_body(u, accs):
        accs = list(accs)
        shift = (u + 97) % 128
        for cb in range(4):
            tile = jnp.concatenate([wuk_v[128 * cb + 32 * i + u] for i in range(4)], axis=0)
            r = pltpu.roll(_nt(qa_b, tile), shift, 1)
            accs[cb] = jnp.where(skew == u, r, accs[cb])
        return tuple(accs)

    accs = lax.fori_loop(0, 32, qabs_body, tuple(jnp.zeros((32, 128), F32) for _ in range(4)))
    qabs_b = jnp.concatenate([_skew_rows(a) for a in accs], axis=1).astype(BF16)

    cp_ckv.wait()
    kc = 512

    def score_body(c, m):
        k0 = pl.multiple_of(c * kc, kc)
        s = _nt(qabs_b, ckv_v[pl.ds(k0, kc), :]) * scale
        s_s[:, pl.ds(k0, kc)] = s
        for j in range(kc // 128):
            m = jnp.maximum(m, s[:, 128 * j:128 * (j + 1)])
        return m

    m = lax.fori_loop(0, SK // kc, score_body, jnp.full((32, 128), -jnp.inf, F32))
    m = jnp.max(m, axis=1, keepdims=True)

    def pv_body(c, carry):
        l, acc = carry
        k0 = pl.multiple_of(c * kc, kc)
        p = jnp.exp(s_s[:, pl.ds(k0, kc)] - m)
        for j in range(kc // 128):
            l = l + p[:, 128 * j:128 * (j + 1)]
        return l, acc + _nn(p.astype(BF16), ckv_v[pl.ds(k0, kc), :])

    l, ctxc = lax.fori_loop(0, SK // kc, pv_body,
                            (jnp.zeros((32, 128), F32), jnp.zeros((32, DC), F32)))
    ctxc = (ctxc / jnp.sum(l, axis=1, keepdims=True)).astype(BF16)
    flip = (_iota((32, 128), 0) + _iota((32, 128), 1) == 31).astype(F32).astype(BF16)
    ctxn = _nn(flip, jnp.concatenate([ctxc, jnp.zeros((96, DC), BF16)], axis=0))
    ctxk = [_skew_rows(ctxn[:, 128 * cb:128 * (cb + 1)]) for cb in range(4)]

    cp_wuv.wait()
    diag = (lane % 32) == row

    def ctx_body(u, acc):
        shift = (128 - u) % 128
        for cb in range(4):
            lhs = jnp.where(diag, pltpu.roll(ctxk[cb], shift, 1), 0.0).astype(BF16)
            tile = jnp.concatenate([wuv_v[128 * cb + 32 * i + u] for i in range(4)], axis=0)
            acc = acc + _nn(lhs, tile)
        return acc

    ctx_b = lax.fori_loop(0, 32, ctx_body, jnp.zeros((32, 128), F32)).astype(BF16)

    cp_bwq.wait()
    xb = jnp.broadcast_to(xf, (QR, M)).astype(BF16)
    for n in range(H * D // 512):
        cols = slice(512 * n, 512 * (n + 1))
        qb_s[:, cols] = _nn(xb, bwq_v[:, cols]).astype(BF16)

    cp_k.wait()

    def head_body(h, carry):
        c0 = pl.multiple_of(h * D, D)
        s = _nt(qb_s[:, pl.ds(c0, D)], k_v[h]) * scale
        p = jnp.exp(s - jnp.max(s, axis=1, keepdims=True))
        o = _nn(p.astype(BF16), v_v[h])
        o_s[:, pl.ds(c0, D)] = (o / jnp.sum(p, axis=1, keepdims=True)).astype(BF16)
        return carry

    for g, (lo, hi) in enumerate(zip(V_SPLIT[:-1], V_SPLIT[1:])):
        cp_v[g].wait()
        lax.fori_loop(lo, hi, head_body, 0)

    cp_wo.wait()
    row16 = _iota((16, 128), 0)
    acc_a = jnp.zeros((16, M), F32)
    for h in range(H):
        grp = ctx_b[16 * (h // 16):16 * (h // 16 + 1), :]
        acc_a = acc_a + _nn(jnp.where(row16 == (h % 16), grp, jnp.zeros_like(grp)), wo_v[h])
    a = jnp.sum(acc_a, axis=0, keepdims=True)

    cp_g.wait()
    gw = gw_v[...].astype(F32).reshape(1, M)
    gate = jax.nn.sigmoid(jnp.sum(xf * gw, axis=1, keepdims=True))

    gate_b = 1.0 - gate
    gb = jnp.broadcast_to(gate_b, (8, M))
    acc_s[...] = jnp.broadcast_to(gate * a, (8, M))
    nt = H * D - TAIL0
    o_rows = jnp.broadcast_to(o_s[0:1, TAIL0:].astype(F32), (128, nt)).astype(BF16)
    eye = (_iota((nt, nt), 0) == _iota((nt, nt), 1)).astype(F32).astype(BF16)
    ocol_s[...] = _nt(eye, o_rows) * gate_b

    for j, (s0, n) in enumerate(BWO_MXU):
        cp_bwo[j].wait()
        part = _nn(o_s[:, s0:s0 + n], bwo_v[s0:s0 + n, :])[0:8, :]
        acc_s[...] = acc_s[...] + gb * part

    sub8 = _iota((8, M), 0)
    accv_s[...] = jnp.where(sub8 == 0, acc_s[...], 0.0)
    for j, (s0, n) in enumerate(BWO_VPU):
        cp_bwo[len(BWO_MXU) + j].wait()
        oc = ocol_s[s0 - TAIL0:s0 - TAIL0 + n, :]
        outs = []
        for t in range(M // 128):
            cols = slice(128 * t, 128 * (t + 1))
            w = bwo_v[s0:s0 + n, cols].astype(F32)
            acc = accv_s[:, cols] + (w * oc).reshape(n // 8, 8, 128).sum(axis=0)
            if j + 1 < len(BWO_VPU):
                accv_s[:, cols] = acc
            else:
                outs.append(jnp.sum(acc, axis=0, keepdims=True))
        if outs:
            out_ref[0] = jnp.concatenate(outs, axis=1).astype(BF16)


@jax.jit
def pallas_gated_mix__compressed_kv_cla__gqa_block_cached__decode_kernel(
    A_x: jax.Array,
    A_c_kv: jax.Array,
    A_w_q: jax.Array,
    A_w_uk: jax.Array,
    A_w_uv: jax.Array,
    A_w_o: jax.Array,
    B_x: jax.Array,
    B_k_cache: jax.Array,
    B_v_cache: jax.Array,
    B_wq: jax.Array,
    B_wo: jax.Array,
    gate_w: jax.Array,
):
    del B_x
    hbm = pl.BlockSpec(memory_space=pl.ANY)
    return pl.pallas_call(
        _kernel,
        out_shape=jax.ShapeDtypeStruct((1, 1, M), BF16),
        in_specs=[hbm] * 11,
        out_specs=pl.BlockSpec(memory_space=pltpu.VMEM),
        scratch_shapes=[
            pltpu.VMEM((1, 1, M), BF16),
            pltpu.VMEM((M,), BF16),
            pltpu.VMEM((SK, DC), BF16),
            pltpu.VMEM((M, H, D), BF16),
            pltpu.VMEM((DC, H, D), BF16),
            pltpu.VMEM((DC, H, D), BF16),
            pltpu.VMEM((H, D, M), BF16),
            pltpu.VMEM((H, SK, D), BF16),
            pltpu.VMEM((H, SK, D), BF16),
            pltpu.VMEM((M, H * D), BF16),
            pltpu.VMEM((H * D, M), BF16),
            pltpu.VMEM((160, 128), F32),
            pltpu.VMEM((32, SK), F32),
            pltpu.VMEM((QR, H * D), BF16),
            pltpu.VMEM((QR, H * D), BF16),
            pltpu.VMEM((8, M), F32),
            pltpu.VMEM((H * D - TAIL0, 128), F32),
            pltpu.VMEM((8, M), F32),
            pltpu.SemaphoreType.DMA((N_SEM,)),
        ],
        compiler_params=pltpu.CompilerParams(
            vmem_limit_bytes=112 * 1024 * 1024,
            disable_semaphore_checks=True,
        ),
    )(A_x, A_c_kv, A_w_q, A_w_uk, A_w_uv, A_w_o, B_k_cache, B_v_cache, B_wq, B_wo, gate_w)
```
